```python
import os as _os
_os.environ.setdefault("JAX_PLATFORMS", "cpu")
import jax
import jax.numpy as jnp

def _softmax(x, axis=-1):
    return jax.nn.softmax(x, axis=axis)
def _gelu(x):
    return jax.nn.gelu(x, approximate=True)
def _silu(x):
    return jax.nn.silu(x)
def _sigmoid(x):
    return jax.nn.sigmoid(x)
def _layernorm(x, axis=-1, eps=1e-5):
    m = jnp.mean(x, axis=axis, keepdims=True)
    v = jnp.var(x, axis=axis, keepdims=True)
    return (x - m) / jnp.sqrt(v + eps)
def _scatter_add(tgt, idx, src, axis=0):
    return tgt.at[idx].add(src)
def _segment_sum(src, seg, n):
    return jax.ops.segment_sum(src, seg, n)
class _Rng:
    def __init__(self, key):
        self._k = key
    def _next(self):
        self._k, sub = jax.random.split(self._k)
        return sub
    def normal(self, shape):
        return jax.random.normal(self._next(), shape, dtype=jnp.bfloat16)
    def randint(self, lo, hi, shape):
        return jax.random.randint(self._next(), shape, lo, hi, dtype=jnp.int32)
    def uniform(self, shape, lo=0.0, hi=1.0):
        return jax.random.uniform(self._next(), shape, jnp.bfloat16, lo, hi)
    def permutation(self, n):
        return jax.random.permutation(self._next(), n)


kernel_name = 'parallel_sum__sliding_local_dilated__glu_gated_reglu__prompt'

def setup_inputs():
    _rng = _Rng(jax.random.key(int.from_bytes(__import__("os").urandom(4), "little")))
    _w = (lambda a: (lambda t: t.astype(jnp.bfloat16) if jnp.issubdtype(t.dtype, jnp.floating) else t)(jnp.asarray(a)))
    def _A_setup():
        B, S, D = 1, 2048, 576
        return {
            "x": _w((lambda *s: _rng.normal(s) * 0.05)(B, S, D)),
            "wqkv": _w((lambda *s: _rng.normal(s) * 0.05)(D, 3 * D)),
            "wo": _w((lambda *s: _rng.normal(s) * 0.05)(D, D)),
        }
    _A_in = _A_setup()

    def _B_setup():
        B, S, D, F = 1, 2048, 576, 4608
        return {
            "x": _w((lambda *s: _rng.normal(s) * 0.05)(B, S, D)),
            "W_gate": _w((lambda *s: _rng.normal(s) * 0.1)(D, F) * (2.0 / D) ** 0.5),
            "W_up": _w((lambda *s: _rng.normal(s) * 0.1)(D, F) * (2.0 / D) ** 0.5),
            "W_down": _w((lambda *s: _rng.normal(s) * 0.1)(F, D) * (1.0 / F) ** 0.5),
        }
    _B_in = _B_setup()

    return {
        "A_x": _A_in["x"],
        "A_wqkv": _A_in["wqkv"],
        "A_wo": _A_in["wo"],
        "B_x": _B_in["x"],
        "B_W_gate": _B_in["W_gate"],
        "B_W_up": _B_in["W_up"],
        "B_W_down": _B_in["W_down"],
    }

def reference(A_x, A_wqkv, A_wo, B_x, B_W_gate, B_W_up, B_W_down):
    def _A_ref(x, wqkv, wo):
        B, S, D = x.shape
        H = 32; Dh = D // H
        W, dil = 8, 2
        qkv = (lambda x, *d: x.transpose(*d))((x @ wqkv).reshape(B, S, 3, H, Dh), 2, 0, 3, 1, 4)
        q, k, v = qkv[0], qkv[1], qkv[2]
        scale = Dh ** -0.5
        pos = jnp.arange(S)
        off = jnp.arange(W) * dil
        idx = pos[:, None] - off[None, :]
        mask = idx >= 0
        idx_c = jnp.where(mask, idx, 0).reshape(-1)
        kg = k[:, :, idx_c, :].reshape(B, H, S, W, Dh)
        vg = v[:, :, idx_c, :].reshape(B, H, S, W, Dh)
        logits = jnp.einsum("bhsd,bhswd->bhsw", q, kg) * scale
        logits = jnp.where(mask[None, None, :, :], logits, -1e9)
        attn = _softmax(logits, axis=-1)
        o = jnp.einsum("bhsw,bhswd->bhsd", attn, vg)
        return (lambda x, *d: x.transpose(*d))(o, 0, 2, 1, 3).reshape(B, S, D) @ wo

    def _B_ref(x, W_gate, W_up, W_down):
        gate = jnp.einsum("bsd,df->bsf", x, W_gate)
        up = jnp.einsum("bsd,df->bsf", x, W_up)
        gate = gate * (lambda x, dt: x.astype(dt))(gate > 0, gate.dtype)
        h = gate * up
        return jnp.einsum("bsf,fd->bsd", h, W_down)

    x = A_x
    xn = _layernorm(x, axis=-1)
    return x + _A_ref(xn, A_wqkv, A_wo) + _B_ref(xn, B_W_gate, B_W_up, B_W_down)
```

```python
import functools
import math

import jax
import jax.numpy as jnp
import numpy as np
from jax import lax
from jax.experimental import pallas as pl
from jax.experimental.pallas import tpu as pltpu

F32 = jnp.float32
BF16 = jnp.bfloat16
U32 = jnp.uint32

HEADS = 32
WINDOW = 8
DILATION = 2
LN_EPS = 1e-5
T = 128
HT = T // 2
HG = 8
R = 16

A7 = (((1, 0), (1, 3)), ((1, 2), (1, 3)), ((1, 0),), ((1, 3),), ((1, 0), (1, 1)), ((1, 2), (-1, 0)), ((1, 1), (-1, 3)))
B7 = (((1, 0), (1, 3)), ((1, 0),), ((1, 1), (-1, 3)), ((1, 2), (-1, 0)), ((1, 3),), ((1, 0), (1, 1)), ((1, 2), (1, 3)))
C7 = (((1, 0), (1, 3), (-1, 4), (1, 6)), ((1, 2), (1, 4)), ((1, 1), (1, 3)), ((1, 0), (-1, 1), (1, 2), (1, 5)))
TAIL = {2: (((1, 0),), 1), 3: (((1, 1),), 0), 5: (((1, 1), (-1, 0)), 1), 6: (((1, 0), (-1, 1)), 0)}
TAILS = sorted(TAIL)

QK_ORDER = (1, 5, 2, 3, 0, 4, 6)
V_ORDER, V_INNER = (3, 0, 4, 6, 2, 1, 5), ('314k2506', 'k1320465')
UP_FIRST_ORDER, UP_FIRST_INNER = (4, 3, 2, 1, 0, 5, 6), ('13064k25', '01k43625')
UP_ORDER, UP_INNER = (4, 2, 3, 0, 1, 5, 6), ('13064k25', '01k34625')
DOWN_ORDER, DOWN_INNER = (2, 3, 1, 0, 4, 5, 6), ('341605k2', '3146k502')


def _lin(terms, get):
    r = get(terms[0][1])
    for sign, key in terms[1:]:
        r = (lax.add if sign > 0 else lax.sub)(r, get(key))
    return r


def _blk(o, i):
    return o // 2 * 2 + i // 2, o % 2 * 2 + i % 2


def _outer(tab, po, get):
    return [_lin(tab[po], lambda o: get(*_blk(o, i))) for i in range(4)]


def _completion(order, p):
    last = [max((q for _, q in terms), key=order.index) for terms in C7]
    return ([o for o in range(4) if last[o] == p],
            any(last[o] != p and q == p for o in range(4) for _, q in C7[o]))


def _combine(product, order, park):
    c, sign, left = [None] * 4, [1] * 4, [len(terms) for terms in C7]
    for p in order:
        if p == 'k':
            for k, o in enumerate((0, 3)):
                if 0 < left[o] < len(C7[o]) - 1:
                    c[o] = park(k, c[o])
            continue
        y = product(int(p))
        for o, s in ((o, s) for o, terms in enumerate(C7) for s, q in terms if q == int(p)):
            left[o] -= 1
            if c[o] is None:
                c[o], sign[o] = y, s
            elif sign[o] < 0:
                c[o], sign[o] = y - c[o], 1
            else:
                c[o] = c[o] + y if s > 0 else c[o] - y
    return c


def _dot(a, b):
    return lax.dot_general(a, b, (((1,), (0,)), ((), ())), preferred_element_type=F32)


def _fold(w1, w2, r1, r2):
    def merge(lo, hi):
        return jnp.where(lax.broadcasted_iota(jnp.int32, lo.shape, 1) < HT, lo, hi)

    n = w2.shape[0]
    pad = w2 if n == w1.shape[0] else jnp.concatenate([w2, jnp.zeros_like(w1[n:])], axis=0)
    return merge(w1, w1 - pad), merge(w2, r2 - r1[:n]), merge(r1, pad)


def _split(m):
    return -(-m // (2 * R)) * R


def _weight_operands(po, pi, quad, tail):
    w = _lin(B7[pi], quad)
    if po in TAIL and pi in TAIL:
        r, n = tail(2 * TAIL[po][1] + TAIL[pi][1]), _split(w.shape[0])
        return [v.astype(BF16) for v in _fold(w[:n], w[n:], r[:n], r[n:])]
    return [w.astype(BF16)]


def _tail_operand(po, pi, tail):
    return _lin(TAIL[po][0], lambda io: _lin(TAIL[pi][0], lambda ii: tail(2 * io + ii)))


def _product(w, x, xr):
    if len(w) == 1:
        return _dot(w[0], x(0, T))
    shared = _dot(w[2], jnp.concatenate([xr(), x(HT, HT)], axis=0))
    return jnp.concatenate([_dot(w[0], x(0, T)) + shared,
                            _dot(w[1], jnp.concatenate([x(0, HT), xr()], axis=0)) + shared[:w[1].shape[0]]], axis=0)


class _Arena:
    def __init__(self):
        self.top = self.size = 0

    def alloc(self, shape, rows):
        base = self.top
        self.top += math.prod(shape) * rows
        self.size = max(self.size, -(-self.top // HT) * HT)

        def row(*idx):
            flat = 0
            for i, n in zip(idx, shape, strict=True):
                flat = flat * n + i % n
            return base + flat * rows
        return row


def _make_kernel(S, D, F):
    DH = D // HEADS
    NG = HEADS // HG
    DQ = D // 4
    TB = FC = 4 * T
    NTB, NIT, NTILE = S // TB, F // FC, S // T
    ATT, ATT0 = divmod(NG * NTILE, NIT)
    scale = float(DH) ** -0.5
    assert D == 4 * T + HT and NG == 4 and DQ == HG * DH and NTB == 4 and S == NTB * TB
    assert F == NIT * FC and NIT > 3 and ATT0 + ATT >= NG

    x_arena, q_arena, f_arena, p_arena = _Arena(), _Arena(), _Arena(), _Arena()
    XS, XR = x_arena.alloc((7, 7), T), x_arena.alloc((4, 4), HT)
    WQ, XQ = q_arena.alloc((7, 2, 3, 2), DQ), q_arena.alloc((7, 2), T)
    UP, UK, UG = f_arena.alloc((2, 2, 4, 7), T), f_arena.alloc((2, 2, 7, 2), T), f_arena.alloc((2, 4, 4), T)
    f_arena.top = 0
    DP, DK, DA, DS, DW = (f_arena.alloc((4, 7), DQ), f_arena.alloc((7, 2), DQ), f_arena.alloc((2, NIT + 1, 4), T),
                          f_arena.alloc((8,), DQ), f_arena.alloc((2, 4), DQ))
    f_arena.top = 0
    TM, TO = f_arena.alloc((5,), 3 * D), f_arena.alloc((5,), D)
    XN, QP, QS = p_arena.alloc((4,), D), p_arena.alloc((2, 4, 7), DQ), p_arena.alloc((4, 2, 2), DQ)
    p_arena.top = 0
    VP, VK = p_arena.alloc((2, 4, 7), DQ), p_arena.alloc((2, 7, 2), DQ)
    assert p_arena.size <= NIT * 16 * T

    def kernel(x_hbm, wqkv_hbm, wo_hbm, wg_hbm, wu_hbm, wd_hbm, o_hbm,
               xo, wqkv, wo, wbuf, xs, wq, wv, wt, wd, wot, tmp, hid, qkv, attn, sem_x, sem_w, sem_a, sem_o):
        ptmp = hid.at[0]

        def load(ref, r0, n):
            if ref.dtype == U32:
                return pltpu.bitcast(ref[pl.ds(r0 // 2, n // 2), :], BF16)
            return ref[pl.ds(r0, n), :]

        def store(ref, r0, y):
            if ref.dtype == U32:
                ref[pl.ds(pl.multiple_of(r0 // 2, R // 2), y.shape[0] // 2), :] = pltpu.bitcast(y.astype(BF16), U32)
            else:
                ref[pl.ds(r0, y.shape[0]), :] = y.astype(ref.dtype)

        def parker(ref, row):
            def park(k, v):
                store(ref, row(k), v)
                return load(ref, row(k), v.shape[0])
            return park

        def k_tile(get, n):
            return get(n * T, T) if n < 4 else jnp.concatenate([get(n * T, HT)] * 2, axis=0)

        def x_copy(t):
            return pltpu.make_async_copy(x_hbm.at[:, pl.ds(t * TB, TB)], xo.at[t], sem_x.at[t])

        w_groups = (0, 9, 3 * NIT)

        def w_start(k):
            for n in range(w_groups[k], w_groups[k + 1]):
                src = (wg_hbm, wu_hbm, wd_hbm)[n % 3]
                pltpu.make_async_copy(src.at[:, pl.ds(n // 3 * FC, FC)], wbuf.at[n], sem_w.at[k]).start()

        def w_wait(k):
            dst = wbuf.at[pl.ds(w_groups[k], w_groups[k + 1] - w_groups[k])]
            pltpu.make_async_copy(dst, dst, sem_w.at[k]).wait()

        def o_start(t, o):
            rs, c0 = pl.ds(o % 2 * 2 * DQ, 2 * DQ), o // 2 * 2 * T
            pltpu.make_async_copy(xo.at[t, rs, pl.ds(c0, 2 * T)],
                                  o_hbm.at[rs, pl.ds(pl.multiple_of(t * TB + c0, 2 * T), 2 * T)], sem_o.at[t]).start()

        def layernorm(t, pairs=(0, 2)):
            rstds = []
            for j in pairs:
                x = xo[t, :, pl.ds(j * T, 2 * T)].astype(F32)
                for i in range(2):
                    u = pltpu.bitcast(xo[t, :, pl.ds((j + i) * T, T)], U32)
                    lo, hi = [lax.bitcast_convert_type(v, F32) for v in (u << 16, u & np.uint32(0xFFFF0000))]
                    d0, d1 = lo - lo[:1], hi - lo[:1]
                    mean = jnp.sum(d0 + d1, axis=0, keepdims=True) * (1.0 / D)
                    var = jnp.sum(d0 * d0 + d1 * d1, axis=0, keepdims=True) * (1.0 / D) - mean * mean
                    rstds.append(lax.rsqrt(var + LN_EPS))
                    store(ptmp, XN(j + i), (x[:, i * T:(i + 1) * T] - (lo[:1] + mean)) * rstds[-1])
            return rstds

        def x_operands(t, po):
            c = _outer(A7, po, lambda j, k: load(ptmp, XN(j) + k * T, T))
            for pi in range(7):
                store(xs.at[t], XS(po, pi), _lin(A7[pi], c.__getitem__))
                if po in TAIL and pi in TAIL:
                    store(xs.at[t], XR(TAILS.index(po), TAILS.index(pi)),
                          _tail_operand(po, pi, lambda j: load(ptmp, XN(j) + 4 * T, HT)))
            for ii in range(2):
                store(wq, XQ(po, ii), c[1 + ii])

        def x_products(t, po, w, order, park, each=lambda y: y):
            return _combine(lambda pi: each(_product(
                w(pi), lambda r, n: load(xs.at[t], XS(po, pi) + r, n),
                lambda: load(xs.at[t], XR(TAILS.index(po), TAILS.index(pi)), HT))), order[po in TAIL], park)

        def transpose_wqkv(c0, c1, tiles):
            for n in tiles:
                store(tmp, TM(n) + c0, k_tile(lambda r, rows: wqkv[pl.ds(r, rows), pl.ds(c0, c1 - c0)], n).T)

        def wqkv_rows(part, ds):
            return lambda n, g: jnp.concatenate(
                [tmp[pl.ds(TM(n) + part * D + g * DQ + d, HG, stride=DH), :] for d in ds], axis=0)

        def wqk_operands(po, part, after):
            get = wqkv_rows(part, range(DH))
            c = _outer(B7, po, get)
            if after is not None:
                c[1] = jnp.where(lax.population_count(lax.bitcast_convert_type(after, jnp.int32)) > 32, 0.0, c[1])
            out = {}
            for n in range(2):
                ops = c[2 * n:2 * n + 2]
                if n == 1 and po in TAIL:
                    ops = _fold(*ops, *[get(4, 2 * TAIL[po][1] + jj) for jj in range(2)])
                for k, y in enumerate(ops):
                    store(wq, WQ(po, n, k, part), y)
                    out[po, n, k] = y
            return out

        def wv_operands(po, s, delay):
            n = _split(DQ)
            both = not isinstance(s, int)
            get = wqkv_rows(2, [r0 // HG + 2 * s + d for r0 in (0, n)[:1 + both] for d in range(2)])
            c = [delay(v) for v in _outer(B7, po, get)]
            for pi in range(7):
                w = _lin(B7[pi], c.__getitem__)
                ops = [w[:R], w[R:] if both else None]
                if po in TAIL and pi in TAIL:
                    r = get(4, 2 * TAIL[po][1] + TAIL[pi][1])
                    ops = _fold(*ops, r[:R], r[R:]) if both else ops + [_fold(w, jnp.zeros_like(w), r, r)[2]]
                for r0, y in zip((0, n, DQ), ops):
                    if y is not None:
                        store(wv.at[7 * po + pi], r0 + s * R, y)

        def put_qkv(t, part, order, po, i, y, row):
            done, later = _completion(order, po)
            if later:
                store(ptmp, row(po), y)
            for o in done:
                j, g = _blk(o, i)
                qkv[(4 * t + j + 1) * NG + g, pl.ds(part * DQ, DQ), :] = _lin(
                    C7[o], lambda q: y if q == po else load(ptmp, row(q), DQ))

        folded = [po for po in QK_ORDER if po in TAIL]

        def folded_pair(po):
            return folded[folded.index(po):][:2] if po in folded[::2] else []

        def project_qk(t, po, lo, hi, each=lambda y: None, fresh=None):
            m = (hi - lo) * DQ

            def w(*idx):
                return fresh[idx].astype(BF16) if fresh else load(wq, WQ(*idx, lo), m)

            def x(po, ii, n, tail_half=None):
                ref, r0 = (xs.at[t], XS(po, 2 + ii)) if n == ii else (wq, XQ(po, ii))
                return jnp.concatenate([load(xs.at[t], XR(TAILS.index(po), ii), HT) if k == tail_half
                                        else load(ref, r0 + k * HT, HT) for k in range(2)], axis=0)

            for q in folded_pair(po):
                for ii in range(2):
                    store(ptmp, QS(TAILS.index(q), ii, lo), _dot(w(q, 1, 2), x(q, ii, 1, 0)))
            for ii in range(2):
                for jj in range(2):
                    y = _dot(w(po, 0, jj), x(po, ii, 0)) + _dot(w(po, 1, jj), x(po, ii, 1, 1 if po in TAIL and jj else None))
                    if po in TAIL:
                        y += load(ptmp, QS(TAILS.index(po), ii, lo), m)
                    each(y)
                    for part in range(lo, hi):
                        put_qkv(t, part, QK_ORDER, po, 2 * ii + jj, y[(part - lo) * DQ:(part - lo + 1) * DQ],
                                lambda q: QP(part, 2 * ii + jj, q))

        def project_v(t, po):
            n = _split(DQ)

            def w(pi):
                rows = ((0, n), (n, DQ - n), (DQ, n)) if po in TAIL and pi in TAIL else ((0, DQ),)
                return [load(wv.at[7 * po + pi], *r) for r in rows]

            for i, y in enumerate(x_products(t, po, w, V_INNER, parker(ptmp, lambda k: VK(t, po, k)))):
                put_qkv(t, 2, V_ORDER, po, i, y, lambda q: VP(t, i, q))

        def transpose_wo():
            for l in range(5):
                cols = min(T, D - l * T)
                v = wo[:, pl.ds(l * T, cols)].astype(F32)
                store(tmp, TO(l), v if cols == T else jnp.concatenate([v, jnp.zeros_like(v)], axis=1))
                v = jnp.concatenate([tmp[pl.ds(TO(l) + g * DQ + d, HG, stride=DH), :]
                                     for g in range(NG) for d in range(DH)], axis=0)[:, :cols]
                for n in range(5):
                    wot[n, pl.ds(l * T, cols), :] = k_tile(lambda r, rows: v[r:r + rows], n).T

        def transpose_gate_up(c):
            for n in range(5):
                for m in range(2):
                    for j in range(4):
                        store(wt.at[m, n, j], 0,
                              k_tile(lambda r, rows: wbuf[3 * c + m, pl.ds(r, rows), pl.ds(j * T, T)], n).T)

        lane = lax.broadcasted_iota(jnp.int32, (HG, T), 1)

        def attention_tile(n, may_be_first):
            g, j = n % NG, n // NG
            q = qkv[n + NG, pl.ds(0, DQ), :]
            kv_prev, kv = qkv[n, pl.ds(DQ, 2 * DQ), :], qkv[n + NG, pl.ds(DQ, 2 * DQ), :]

            def window(r):
                prev, cur = kv_prev[r:r + HG], kv[r:r + HG]
                return [cur] + [pltpu.roll(lax.select(lane >= T - w * DILATION, prev, cur), w * DILATION, 1)
                                for w in range(1, WINDOW)]

            logits = None
            for r in range(0, DQ, HG):
                terms = [lax.mul(q[r:r + HG], k) for k in window(r)]
                logits = terms if logits is None else [lax.add(a, b) for a, b in zip(logits, terms)]
            logits = [s * scale for s in logits]
            if may_be_first:
                pos = lane + j * T
                logits = [jnp.where(pos >= w * DILATION, s, -1e9) if w else s for w, s in enumerate(logits)]
            top = functools.reduce(jnp.maximum, logits)
            p = [jnp.exp(s - top) for s in logits]
            inv = 1.0 / functools.reduce(lax.add, p)
            p = [e * inv for e in p]
            out = [functools.reduce(lax.add, [lax.mul(a, v) for a, v in zip(p, window(DQ + r))])
                   for r in range(0, DQ, HG)]
            store(attn.at[j], g * DQ, jnp.concatenate(out, axis=0))

        c1 = 5 * T
        pieces = [(pl.ds(0, 2 * T), pl.ds(0, c1)), (pl.ds(2 * T, D - 2 * T), pl.ds(0, c1)),
                  (pl.ds(0, D), pl.ds(c1, 2 * D - c1)), (pl.ds(0, D), pl.ds(2 * D, D))]
        wq0_copy, wq1_copy, wk_copy, wv_copy = [
            pltpu.make_async_copy(wqkv_hbm.at[ix], wqkv.at[ix], sem_a.at[k]) for k, ix in enumerate(pieces)]
        wo_copy = pltpu.make_async_copy(wo_hbm, wo, sem_a.at[4])
        x0_copies = [pltpu.make_async_copy(x_hbm.at[:, pl.ds(j * T, 2 * T)], xo.at[0, :, pl.ds(j * T, 2 * T)], sem)
                     for j, sem in ((0, sem_x.at[0]), (2, sem_a.at[5]))]
        for c in x0_copies:
            c.start()
        wq0_copy.start()
        for k, c in enumerate(x0_copies):
            c.wait()
            if k == 0:
                wq1_copy.start()
            layernorm(0, [2 * k])
        wq0_copy.wait()
        wk_copy.start()
        x_copy(1).start()
        transpose_wqkv(0, c1, range(2))
        for po in QK_ORDER[:2]:
            x_operands(0, po)
        wq1_copy.wait()
        wv_copy.start()
        transpose_wqkv(0, c1, range(2, 5))
        for po in QK_ORDER[2:]:
            x_operands(0, po)
        for part in range(2):
            fresh = {}
            for k, po in enumerate(QK_ORDER):
                if (part, k) == (0, 6):
                    wk_copy.wait()
                    x_copy(1).wait()
                    x_copy(2).start()
                    x_copy(3).start()
                    transpose_wqkv(c1, 2 * D, range(5))
                    rstds = dict(zip((0, 2, 3, 4), layernorm(1)))
                if (part, k) == (1, 5):
                    wv_copy.wait()
                    transpose_wqkv(2 * D, 3 * D, range(5))
                for q in folded_pair(po) if po in TAIL else [po]:
                    fresh.update(wqk_operands(q, part, rstds.get(QK_ORDER.index(q)) if part else None))
                project_qk(0, po, part, part + 1, fresh=fresh)
        x_copy(2).wait()
        x_copy(3).wait()
        wo_copy.start()
        w_start(0)

        def qk_step(t, carry):
            jobs = [None] * 2 + [(po, s) for po in QK_ORDER for s in (t - 1, jnp.minimum(t + 2, 3), 4)]

            def each(y):
                job = jobs.pop(0) if jobs else None
                if job:
                    r = len(jobs) % 2 * DQ
                    wv_operands(*job, lambda v: jnp.where(t < 0, y[r:r + v.shape[0]], v))

            for po in QK_ORDER:
                x_operands(t, po)
            for po in QK_ORDER:
                project_qk(t, po, 0, 2, each)
            assert not jobs
            layernorm(jnp.minimum(t + 1, NTB - 1))
            return carry

        lax.fori_loop(1, NTB, qk_step, 0)
        w_wait(0)
        wo_copy.wait()
        w_start(1)
        for t in range(NTB):
            for po in V_ORDER:
                project_v(t, po)
            if t == 0:
                rs = pl.ds(DQ, 2 * DQ)
                for g in range(NG):
                    qkv[g, rs, :] = jnp.broadcast_to(qkv[NG + g, rs, pl.ds(0, 1)], (2 * DQ, T))
        transpose_wo()
        transpose_gate_up(0)
        for n in range(ATT0):
            attention_tile(n, n < NG)

        def up_step(it, carry):
            @pl.when(it == w_groups[1] // 3 - 1)
            def _():
                w_wait(1)

            jobs = [(po, r) for po in range(7) for r in range(0, DQ, R)]
            count = [0]

            def down_operands(y):
                count[0] += 1
                if jobs and count[0] >= 96 and count[0] % 2 == 0:
                    po, r = jobs.pop(0)
                    pair = functools.cache(
                        lambda j, n: wbuf[3 * it + 2, pl.ds(j * DQ + r, R), pl.ds(n * 2 * T, 2 * T)].astype(F32))
                    c = _outer(B7, po, lambda n, j: pair(j, n // 2)[:, n % 2 * T:(n % 2 + 1) * T])
                    c = [jnp.where(it < 0, y[:R], v) for v in c]
                    for pi in range(7):
                        store(wd.at[it], (7 * po + pi) * DQ + r, _lin(B7[pi], c.__getitem__))
                return y

            out = hid.at[:, pl.ds(pl.multiple_of(it * 16 * T, 16 * T), 16 * T)]
            w = {}
            for t in range(NTB):
                order, inner = (UP_ORDER, UP_INNER) if t else (UP_FIRST_ORDER, UP_FIRST_INNER)
                for m in range(2):
                    for po in order:
                        if t == 0:
                            def get(n, j):
                                return load(wt.at[m, n, j], 0, T).astype(F32)

                            c = _outer(B7, po, get)
                            w[m, po] = [_weight_operands(po, pi, c.__getitem__, functools.partial(get, 4))
                                        for pi in range(7)]
                        c = x_products(t, po, w[m, po].__getitem__, inner,
                                       parker(tmp, lambda k: UK(t, m, po, k)), down_operands)
                        done, later = _completion(order, po)
                        for i, v in enumerate(c):
                            if later:
                                store(tmp, UP(t, m, i, po), v)
                            for o in done:
                                y = _lin(C7[o], lambda q: v if q == po else load(tmp, UP(t, m, i, q), T))
                                if m == 0:
                                    store(tmp, UG(t, o, i), jnp.maximum(y, 0.0))
                                else:
                                    j, k = _blk(o, i)
                                    out[t, pl.ds((4 * j + k) * T, T), :] = load(tmp, UG(t, o, i), T) * y
            assert not jobs
            for k in range(ATT):
                attention_tile(ATT0 + it * ATT + k, ATT0 + k < NG)
            transpose_gate_up(jnp.minimum(it + 1, NIT - 1))
            return carry

        def down_step(t, carry):
            def source(c):
                if c < NIT:
                    return lambda j, k: hid[t, pl.ds((16 * c + 4 * j + k) * T, T), :]
                return lambda j, k: load(attn.at[4 * t + j], k * T, T if k < 4 else HT).astype(F32)

            count = [0]
            for n, po in enumerate(DOWN_ORDER):
                staged = [len(A7[po]) > 1] * NIT + [True]
                for c in range(NIT + 1):
                    if staged[c]:
                        for i, v in enumerate(_outer(A7, po, source(c))):
                            store(tmp, DA(n, c, i), v)
                for i, v in enumerate(_outer(B7, po, lambda k, j: wot[k, pl.ds(j * DQ, DQ), :])):
                    store(tmp, DW(n, i), v)
                done, later = _completion(DOWN_ORDER, po)

                def product(pi):
                    if po == DOWN_ORDER[-1] and pi == int(DOWN_INNER[po in TAIL].replace('k', '')[3]):
                        for o in range(4):
                            if o not in done:
                                o_start(t, o)

                    def x(c, r=0, rows=T):
                        return _lin(A7[pi], lambda i: load(tmp, DA(n, c, i) + r, rows) if staged[c]
                                    else source(c)(*_blk(A7[po][0][1], i))).astype(BF16)

                    y = None
                    for c in range(NIT):
                        v = _dot(load(wd.at[c], (7 * po + pi) * DQ, DQ), x(c))
                        y = v if y is None else y + v
                        count[0] += 1
                        if count[0] % 4 == 0:
                            y = parker(tmp, DS)(count[0] // 4, y)
                    count[0] += 1
                    w = _weight_operands(po, pi, lambda i: load(tmp, DW(n, i), DQ),
                                         lambda j: wot[4, pl.ds(j * DQ, DQ), :])
                    return y + _product(w, functools.partial(x, NIT),
                                        lambda: _tail_operand(po, pi, lambda j: source(NIT)(j, 4)).astype(BF16))

                c = _combine(product, DOWN_INNER[po in TAIL], parker(tmp, lambda k: DK(po, k)))
                if later:
                    for i, v in enumerate(c):
                        store(tmp, DP(i, po), v)
                for o in done:
                    for jj in range(2):
                        y = [_lin(C7[o], lambda q: c[i] if q == po else load(tmp, DP(i, q), DQ)) for i in (jj, 2 + jj)]
                        ix = (t, pl.ds((o % 2 * 2 + jj) * DQ, DQ), pl.ds(o // 2 * 2 * T, 2 * T))
                        xo[ix] = (jnp.concatenate(y, axis=1) + xo[ix].astype(F32)).astype(BF16)
            for o in done:
                o_start(t, o)
            return carry

        lax.fori_loop(0, NIT, up_step, 0)
        lax.fori_loop(0, NTB, down_step, 0)
        for t in range(NTB):
            pltpu.make_async_copy(xo.at[t], xo.at[t], sem_o.at[t]).wait()

    scratch = [
        pltpu.VMEM((NTB, D, TB), BF16),
        pltpu.VMEM((D, 3 * D), BF16),
        pltpu.VMEM((D, D), BF16),
        pltpu.VMEM((3 * NIT, D, FC), BF16),
        pltpu.VMEM((NTB, x_arena.size // 2, T), U32),
        pltpu.VMEM((q_arena.size // 2, T), U32),
        pltpu.VMEM((50, (DQ + _split(DQ)) // 2, T), U32),
        pltpu.VMEM((2, 5, 4, HT, T), U32),
        pltpu.VMEM((NIT, 52 * DQ // 2, T), U32),
        pltpu.VMEM((5, D, T), F32),
        pltpu.VMEM((f_arena.size, T), F32),
        pltpu.VMEM((NTB, NIT * 16 * T, T), F32),
        pltpu.VMEM(((NTILE + 1) * NG, -(-3 * DQ // 32) * 32, T), F32),
        pltpu.VMEM((NTILE, D // 2, T), U32),
        pltpu.SemaphoreType.DMA((NTB,)),
        pltpu.SemaphoreType.DMA((2,)),
        pltpu.SemaphoreType.DMA((6,)),
        pltpu.SemaphoreType.DMA((NTB,)),
    ]
    return kernel, scratch


@jax.jit
def pallas_parallel_sum__sliding_local_dilated__glu_gated_reglu__prompt_kernel(
    A_x: jax.Array,
    A_wqkv: jax.Array,
    A_wo: jax.Array,
    B_x: jax.Array,
    B_W_gate: jax.Array,
    B_W_up: jax.Array,
    B_W_down: jax.Array,
):
    del B_x
    B, S, D = A_x.shape
    kernel, scratch = _make_kernel(S, D, B_W_gate.shape[1])
    hbm = pl.BlockSpec(memory_space=pl.ANY)
    out = pl.pallas_call(
        kernel,
        out_shape=jax.ShapeDtypeStruct((D, S), A_x.dtype),
        in_specs=[hbm] * 6,
        out_specs=hbm,
        scratch_shapes=scratch,
        compiler_params=pltpu.CompilerParams(vmem_limit_bytes=127 * 2**20),
        name="fused_block",
    )(A_x.reshape(S, D).T, A_wqkv, A_wo, B_W_gate, B_W_up, B_W_down.T)
    return out.T.reshape(B, S, D)
```

```python
import functools
import math

import jax
import jax.numpy as jnp
import numpy as np
from jax import lax
from jax.experimental import pallas as pl
from jax.experimental.pallas import tpu as pltpu

F32 = jnp.float32
BF16 = jnp.bfloat16
U32 = jnp.uint32

HEADS = 32
WINDOW = 8
DILATION = 2
LN_EPS = 1e-5
T = 128
HT = T // 2
HG = 8
R = 16

A7 = (((1, 0), (1, 3)), ((1, 2), (1, 3)), ((1, 0),), ((1, 3),), ((1, 0), (1, 1)), ((1, 2), (-1, 0)), ((1, 1), (-1, 3)))
B7 = (((1, 0), (1, 3)), ((1, 0),), ((1, 1), (-1, 3)), ((1, 2), (-1, 0)), ((1, 3),), ((1, 0), (1, 1)), ((1, 2), (1, 3)))
C7 = (((1, 0), (1, 3), (-1, 4), (1, 6)), ((1, 2), (1, 4)), ((1, 1), (1, 3)), ((1, 0), (-1, 1), (1, 2), (1, 5)))
TAIL = {2: (((1, 0),), 1), 3: (((1, 1),), 0), 5: (((1, 1), (-1, 0)), 1), 6: (((1, 0), (-1, 1)), 0)}
TAILS = sorted(TAIL)

QK_ORDER = (1, 5, 2, 3, 0, 4, 6)
V_ORDER, V_INNER = (3, 0, 4, 6, 2, 1, 5), ('314k2506', 'k1320465')
UP_FIRST_ORDER, UP_FIRST_INNER = (4, 3, 2, 1, 0, 5, 6), ('13064k25', '01k43625')
UP_ORDER, UP_INNER = (4, 1, 3, 2, 0, 5, 6), ('120364k5', '01k34625')
DOWN_ORDER, DOWN_INNER = (2, 3, 1, 0, 4, 5, 6), ('341605k2', '3146k502')


def _lin(terms, get):
    r = get(terms[0][1])
    for sign, key in terms[1:]:
        r = (lax.add if sign > 0 else lax.sub)(r, get(key))
    return r


def _blk(o, i):
    return o // 2 * 2 + i // 2, o % 2 * 2 + i % 2


def _outer(tab, po, get):
    return [_lin(tab[po], lambda o: get(*_blk(o, i))) for i in range(4)]


def _completion(order, p):
    last = [max((q for _, q in terms), key=order.index) for terms in C7]
    return ([o for o in range(4) if last[o] == p],
            any(last[o] != p and q == p for o in range(4) for _, q in C7[o]))


def _combine(product, order, park):
    c, sign, left = [None] * 4, [1] * 4, [len(terms) for terms in C7]
    for p in order:
        if p == 'k':
            for k, o in enumerate((0, 3)):
                if 0 < left[o] < len(C7[o]) - 1:
                    c[o] = park(k, c[o])
            continue
        y = product(int(p))
        for o, s in ((o, s) for o, terms in enumerate(C7) for s, q in terms if q == int(p)):
            left[o] -= 1
            if c[o] is None:
                c[o], sign[o] = y, s
            elif sign[o] < 0:
                c[o], sign[o] = y - c[o], 1
            else:
                c[o] = c[o] + y if s > 0 else c[o] - y
    return c


def _dot(a, b):
    return lax.dot_general(a, b, (((1,), (0,)), ((), ())), preferred_element_type=F32)


def _fold(w1, w2, r1, r2):
    def merge(lo, hi):
        return jnp.where(lax.broadcasted_iota(jnp.int32, lo.shape, 1) < HT, lo, hi)

    n = w2.shape[0]
    pad = w2 if n == w1.shape[0] else jnp.concatenate([w2, jnp.zeros_like(w1[n:])], axis=0)
    return merge(w1, w1 - pad), merge(w2, r2 - r1[:n]), merge(r1, pad)


def _split(m):
    return -(-m // (2 * R)) * R


def _weight_operands(po, pi, quad, tail):
    w = _lin(B7[pi], quad)
    if po in TAIL and pi in TAIL:
        r, n = tail(2 * TAIL[po][1] + TAIL[pi][1]), _split(w.shape[0])
        return [v.astype(BF16) for v in _fold(w[:n], w[n:], r[:n], r[n:])]
    return [w.astype(BF16)]


def _tail_operand(po, pi, tail):
    return _lin(TAIL[po][0], lambda io: _lin(TAIL[pi][0], lambda ii: tail(2 * io + ii)))


def _product(w, x, xr):
    if len(w) == 1:
        return _dot(w[0], x(0, T))
    shared = _dot(w[2], jnp.concatenate([xr(), x(HT, HT)], axis=0))
    return jnp.concatenate([_dot(w[0], x(0, T)) + shared,
                            _dot(w[1], jnp.concatenate([x(0, HT), xr()], axis=0)) + shared[:w[1].shape[0]]], axis=0)


class _Arena:
    def __init__(self):
        self.top = self.size = 0

    def alloc(self, shape, rows):
        base = self.top
        self.top += math.prod(shape) * rows
        self.size = max(self.size, -(-self.top // HT) * HT)

        def row(*idx):
            flat = 0
            for i, n in zip(idx, shape, strict=True):
                flat = flat * n + i % n
            return base + flat * rows
        return row


def _make_kernel(S, D, F):
    DH = D // HEADS
    NG = HEADS // HG
    DQ = D // 4
    TB = FC = 4 * T
    NTB, NIT, NTILE = S // TB, F // FC, S // T
    ATT, ATT0 = divmod(NG * NTILE, NIT)
    scale = float(DH) ** -0.5
    assert D == 4 * T + HT and NG == 4 and DQ == HG * DH and NTB == 4 and S == NTB * TB
    assert F == NIT * FC and NIT > 3 and ATT0 + ATT >= NG

    x_arena, q_arena, f_arena, p_arena = _Arena(), _Arena(), _Arena(), _Arena()
    XS, XR = x_arena.alloc((7, 7), T), x_arena.alloc((4, 4), HT)
    WQ, XQ = q_arena.alloc((7, 2, 3, 2), DQ), q_arena.alloc((7, 2), T)
    UP, UK, UG = f_arena.alloc((2, 2, 4, 7), T), f_arena.alloc((2, 2, 7, 2), T), f_arena.alloc((2, 4, 4), T)
    f_arena.top = 0
    DP, DK, DA, DS, DW = (f_arena.alloc((4, 7), DQ), f_arena.alloc((7, 2), DQ), f_arena.alloc((2, 4, NIT + 1), T),
                          f_arena.alloc((8,), DQ), f_arena.alloc((2, 4), DQ))
    f_arena.top = 0
    TM, TO = f_arena.alloc((5,), 3 * D), f_arena.alloc((5,), D)
    XN, QP, QS = p_arena.alloc((4,), D), p_arena.alloc((2, 4, 7), DQ), p_arena.alloc((4, 2, 2), DQ)
    p_arena.top = 0
    VP, VK = p_arena.alloc((2, 4, 7), DQ), p_arena.alloc((2, 7, 2), DQ)
    assert p_arena.size <= NIT * 16 * T

    def kernel(x_hbm, wqkv_hbm, wo_hbm, wg_hbm, wu_hbm, wd_hbm, o_hbm,
               xo, wqkv, wo, wbuf, xs, wq, wv, wt, wd, wot, tmp, hid, qkv, attn, sem_x, sem_w, sem_a, sem_o):
        ptmp = hid.at[0]

        def load(ref, r0, n):
            if ref.dtype == U32:
                return pltpu.bitcast(ref[pl.ds(r0 // 2, n // 2), :], BF16)
            return ref[pl.ds(r0, n), :]

        def store(ref, r0, y):
            if ref.dtype == U32:
                ref[pl.ds(pl.multiple_of(r0 // 2, R // 2), y.shape[0] // 2), :] = pltpu.bitcast(y.astype(BF16), U32)
            else:
                ref[pl.ds(r0, y.shape[0]), :] = y.astype(ref.dtype)

        def parker(ref, row):
            def park(k, v):
                store(ref, row(k), v)
                return load(ref, row(k), v.shape[0])
            return park

        def k_tile(get, n):
            return get(n * T, T) if n < 4 else jnp.concatenate([get(n * T, HT)] * 2, axis=0)

        def x_copy(t):
            return pltpu.make_async_copy(x_hbm.at[:, pl.ds(t * TB, TB)], xo.at[t], sem_x.at[t])

        w_groups = (0, 9, 3 * NIT)

        def w_start(k):
            for n in range(w_groups[k], w_groups[k + 1]):
                src = (wg_hbm, wu_hbm, wd_hbm)[n % 3]
                pltpu.make_async_copy(src.at[:, pl.ds(n // 3 * FC, FC)], wbuf.at[n], sem_w.at[k]).start()

        def w_wait(k):
            dst = wbuf.at[pl.ds(w_groups[k], w_groups[k + 1] - w_groups[k])]
            pltpu.make_async_copy(dst, dst, sem_w.at[k]).wait()

        def o_start(t, o):
            rs, c0 = pl.ds(o % 2 * 2 * DQ, 2 * DQ), o // 2 * 2 * T
            pltpu.make_async_copy(xo.at[t, rs, pl.ds(c0, 2 * T)],
                                  o_hbm.at[rs, pl.ds(pl.multiple_of(t * TB + c0, 2 * T), 2 * T)], sem_o.at[t]).start()

        def layernorm(t, pairs=(0, 2)):
            rstds = []
            for j in pairs:
                x = xo[t, :, pl.ds(j * T, 2 * T)].astype(F32)
                for i in range(2):
                    u = pltpu.bitcast(xo[t, :, pl.ds((j + i) * T, T)], U32)
                    lo, hi = [lax.bitcast_convert_type(v, F32) for v in (u << 16, u & np.uint32(0xFFFF0000))]
                    d0, d1 = lo - lo[:1], hi - lo[:1]
                    mean = jnp.sum(d0 + d1, axis=0, keepdims=True) * (1.0 / D)
                    var = jnp.sum(d0 * d0 + d1 * d1, axis=0, keepdims=True) * (1.0 / D) - mean * mean
                    rstds.append(lax.rsqrt(var + LN_EPS))
                    store(ptmp, XN(j + i), (x[:, i * T:(i + 1) * T] - (lo[:1] + mean)) * rstds[-1])
            return rstds

        def x_operands(t, po):
            c = _outer(A7, po, lambda j, k: load(ptmp, XN(j) + k * T, T))
            for pi in range(7):
                store(xs.at[t], XS(po, pi), _lin(A7[pi], c.__getitem__))
                if po in TAIL and pi in TAIL:
                    store(xs.at[t], XR(TAILS.index(po), TAILS.index(pi)),
                          _tail_operand(po, pi, lambda j: load(ptmp, XN(j) + 4 * T, HT)))
            for ii in range(2):
                store(wq, XQ(po, ii), c[1 + ii])

        def x_products(t, po, w, order, park, each=lambda y: y):
            x = xs[t, pl.ds(XS(po, 0) // 2, 7 * T // 2), :]
            xr = xs[t, pl.ds(XR(TAILS.index(po), 0) // 2, 4 * HT // 2), :] if po in TAIL else None

            def rows(v, r0, n):
                return pltpu.bitcast(v[r0 // 2:(r0 + n) // 2], BF16)

            return _combine(lambda pi: each(_product(
                w(pi), lambda r, n: rows(x, pi * T + r, n),
                lambda: rows(xr, TAILS.index(pi) * HT, HT))), order[po in TAIL], park)

        def transpose_wqkv(c0, c1, tiles):
            for n in tiles:
                store(tmp, TM(n) + c0, k_tile(lambda r, rows: wqkv[pl.ds(r, rows), pl.ds(c0, c1 - c0)], n).T)

        def wqkv_rows(part, ds):
            return lambda n, g: jnp.concatenate(
                [tmp[pl.ds(TM(n) + part * D + g * DQ + d, HG, stride=DH), :] for d in ds], axis=0)

        def wqk_operands(po, part, after):
            get = wqkv_rows(part, range(DH))
            c = _outer(B7, po, get)
            if after is not None:
                c[1] = jnp.where(lax.population_count(lax.bitcast_convert_type(after, jnp.int32)) > 32, 0.0, c[1])
            out = {}
            for n in range(2):
                ops = c[2 * n:2 * n + 2]
                if n == 1 and po in TAIL:
                    ops = _fold(*ops, *[get(4, 2 * TAIL[po][1] + jj) for jj in range(2)])
                for k, y in enumerate(ops):
                    store(wq, WQ(po, n, k, part), y)
                    out[po, n, k] = y
            return out

        def wv_operands(po, s, delay):
            n = _split(DQ)
            both = not isinstance(s, int)
            get = wqkv_rows(2, [r0 // HG + 2 * s + d for r0 in (0, n)[:1 + both] for d in range(2)])
            c = [delay(v) for v in _outer(B7, po, get)]
            for pi in range(7):
                w = _lin(B7[pi], c.__getitem__)
                ops = [w[:R], w[R:] if both else None]
                if po in TAIL and pi in TAIL:
                    r = get(4, 2 * TAIL[po][1] + TAIL[pi][1])
                    ops = _fold(*ops, r[:R], r[R:]) if both else ops + [_fold(w, jnp.zeros_like(w), r, r)[2]]
                for r0, y in zip((0, n, DQ), ops):
                    if y is not None:
                        store(wv.at[7 * po + pi], r0 + s * R, y)

        def put_qkv(t, part, order, po, i, y, row):
            done, later = _completion(order, po)
            if later:
                store(ptmp, row(po), y)
            for o in done:
                j, g = _blk(o, i)
                qkv[(4 * t + j + 1) * NG + g, pl.ds(part * DQ, DQ), :] = _lin(
                    C7[o], lambda q: y if q == po else load(ptmp, row(q), DQ))

        folded = [po for po in QK_ORDER if po in TAIL]

        def folded_pair(po):
            return folded[folded.index(po):][:2] if po in folded[::2] else []

        def project_qk(t, po, lo, hi, each=lambda y: None, fresh=None):
            m = (hi - lo) * DQ

            def w(*idx):
                return fresh[idx].astype(BF16) if fresh else load(wq, WQ(*idx, lo), m)

            def x(po, ii, n, tail_half=None):
                ref, r0 = (xs.at[t], XS(po, 2 + ii)) if n == ii else (wq, XQ(po, ii))
                return jnp.concatenate([load(xs.at[t], XR(TAILS.index(po), ii), HT) if k == tail_half
                                        else load(ref, r0 + k * HT, HT) for k in range(2)], axis=0)

            for q in folded_pair(po):
                for ii in range(2):
                    store(ptmp, QS(TAILS.index(q), ii, lo), _dot(w(q, 1, 2), x(q, ii, 1, 0)))
            for ii in range(2):
                for jj in range(2):
                    y = _dot(w(po, 0, jj), x(po, ii, 0)) + _dot(w(po, 1, jj), x(po, ii, 1, 1 if po in TAIL and jj else None))
                    if po in TAIL:
                        y += load(ptmp, QS(TAILS.index(po), ii, lo), m)
                    each(y)
                    for part in range(lo, hi):
                        put_qkv(t, part, QK_ORDER, po, 2 * ii + jj, y[(part - lo) * DQ:(part - lo + 1) * DQ],
                                lambda q: QP(part, 2 * ii + jj, q))

        def project_v(t, po):
            n = _split(DQ)

            def w(pi):
                rows = ((0, n), (n, DQ - n), (DQ, n)) if po in TAIL and pi in TAIL else ((0, DQ),)
                return [load(wv.at[7 * po + pi], *r) for r in rows]

            for i, y in enumerate(x_products(t, po, w, V_INNER, parker(ptmp, lambda k: VK(t, po, k)))):
                put_qkv(t, 2, V_ORDER, po, i, y, lambda q: VP(t, i, q))

        def transpose_wo():
            for l in range(5):
                cols = min(T, D - l * T)
                v = wo[:, pl.ds(l * T, cols)].astype(F32)
                store(tmp, TO(l), v if cols == T else jnp.concatenate([v, jnp.zeros_like(v)], axis=1))
                v = jnp.concatenate([tmp[pl.ds(TO(l) + g * DQ + d, HG, stride=DH), :]
                                     for g in range(NG) for d in range(DH)], axis=0)[:, :cols]
                for n in range(5):
                    wot[n, pl.ds(l * T, cols), :] = k_tile(lambda r, rows: v[r:r + rows], n).T

        def transpose_gate_up(c):
            for n in range(5):
                for m in range(2):
                    for j in range(4):
                        store(wt.at[m, n, j], 0,
                              k_tile(lambda r, rows: wbuf[3 * c + m, pl.ds(r, rows), pl.ds(j * T, T)], n).T)

        lane = lax.broadcasted_iota(jnp.int32, (HG, T), 1)

        def attention_tile(n, may_be_first):
            g, j = n % NG, n // NG
            q = qkv[n + NG, pl.ds(0, DQ), :]
            kv_prev, kv = qkv[n, pl.ds(DQ, 2 * DQ), :], qkv[n + NG, pl.ds(DQ, 2 * DQ), :]
            wraps = [lane >= T - w * DILATION for w in range(WINDOW)]

            def window(r):
                prev, cur = kv_prev[r:r + HG], kv[r:r + HG]
                return [cur] + [pltpu.roll(lax.select(wraps[w], prev, cur), w * DILATION, 1)
                                for w in range(1, WINDOW)]

            logits = functools.reduce(lax.add, [
                jnp.concatenate([q[r:r + HG]] * WINDOW, axis=0) * jnp.concatenate(window(r), axis=0)
                for r in range(0, DQ, HG)]) * scale
            logits = [logits[w * HG:(w + 1) * HG] for w in range(WINDOW)]
            if may_be_first:
                pos = lane + j * T
                logits = [jnp.where(pos >= w * DILATION, s, -1e9) if w else s for w, s in enumerate(logits)]
            top = functools.reduce(jnp.maximum, logits)
            p = [jnp.exp(s - top) for s in logits]
            inv = 1.0 / functools.reduce(lax.add, p)
            p = [e * inv for e in p]
            v = zip(*[window(DQ + r) for r in range(0, DQ, HG)])
            store(attn.at[j], g * DQ, functools.reduce(lax.add, [
                jnp.concatenate([pw] * DH, axis=0) * jnp.concatenate(vw, axis=0) for pw, vw in zip(p, v)]))

        c1 = 5 * T
        pieces = [(pl.ds(0, 2 * T), pl.ds(0, c1)), (pl.ds(2 * T, D - 2 * T), pl.ds(0, c1)),
                  (pl.ds(0, D), pl.ds(c1, 2 * D - c1)), (pl.ds(0, D), pl.ds(2 * D, D))]
        wq0_copy, wq1_copy, wk_copy, wv_copy = [
            pltpu.make_async_copy(wqkv_hbm.at[ix], wqkv.at[ix], sem_a.at[k]) for k, ix in enumerate(pieces)]
        wo_copy = pltpu.make_async_copy(wo_hbm, wo, sem_a.at[4])
        x0_copies = [pltpu.make_async_copy(x_hbm.at[:, pl.ds(j * T, 2 * T)], xo.at[0, :, pl.ds(j * T, 2 * T)], sem)
                     for j, sem in ((0, sem_x.at[0]), (2, sem_a.at[5]))]
        for c in x0_copies:
            c.start()
        wq0_copy.start()
        for k, c in enumerate(x0_copies):
            c.wait()
            if k == 0:
                wq1_copy.start()
            layernorm(0, [2 * k])
        wq0_copy.wait()
        wk_copy.start()
        x_copy(1).start()
        transpose_wqkv(0, c1, range(2))
        for po in QK_ORDER[:2]:
            x_operands(0, po)
        wq1_copy.wait()
        wv_copy.start()
        transpose_wqkv(0, c1, range(2, 5))
        for po in QK_ORDER[2:]:
            x_operands(0, po)
        for part in range(2):
            fresh = {}
            for k, po in enumerate(QK_ORDER):
                if (part, k) == (0, 6):
                    wk_copy.wait()
                    x_copy(1).wait()
                    x_copy(2).start()
                    x_copy(3).start()
                    transpose_wqkv(c1, 2 * D, range(5))
                    rstds = dict(zip((0, 2, 3, 4), layernorm(1)))
                if (part, k) == (1, 5):
                    wv_copy.wait()
                    transpose_wqkv(2 * D, 3 * D, range(5))
                for q in folded_pair(po) if po in TAIL else [po]:
                    fresh.update(wqk_operands(q, part, rstds.get(QK_ORDER.index(q)) if part else None))
                project_qk(0, po, part, part + 1, fresh=fresh)
        x_copy(2).wait()
        x_copy(3).wait()
        wo_copy.start()
        w_start(0)

        def qk_step(t, carry):
            jobs = [None] * 2 + [(po, s) for po in QK_ORDER for s in (t - 1, jnp.minimum(t + 2, 3), 4)]

            def each(y):
                job = jobs.pop(0) if jobs else None
                if job:
                    r = len(jobs) % 2 * DQ
                    wv_operands(*job, lambda v: jnp.where(t < 0, y[r:r + v.shape[0]], v))

            for po in QK_ORDER:
                x_operands(t, po)
            for po in QK_ORDER:
                project_qk(t, po, 0, 2, each)
            assert not jobs
            layernorm(jnp.minimum(t + 1, NTB - 1))
            return carry

        lax.fori_loop(1, NTB, qk_step, 0)
        w_wait(0)
        wo_copy.wait()
        w_start(1)
        for t in range(NTB):
            for po in V_ORDER:
                project_v(t, po)
            if t == 0:
                rs = pl.ds(DQ, 2 * DQ)
                for g in range(NG):
                    qkv[g, rs, :] = jnp.broadcast_to(qkv[NG + g, rs, pl.ds(0, 1)], (2 * DQ, T))
        transpose_wo()
        transpose_gate_up(0)
        for n in range(ATT0):
            attention_tile(n, n < NG)

        def up_step(it, carry):
            @pl.when(it == w_groups[1] // 3 - 1)
            def _():
                w_wait(1)

            jobs = [(po, r) for po in range(7) for r in range(0, DQ, R)]
            count = [0]

            def down_operands(y):
                count[0] += 1
                if jobs and count[0] >= 96 and count[0] % 2 == 0:
                    po, r = jobs.pop(0)
                    pair = functools.cache(
                        lambda j, n: wbuf[3 * it + 2, pl.ds(j * DQ + r, R), pl.ds(n * 2 * T, 2 * T)].astype(F32))
                    c = _outer(B7, po, lambda n, j: pair(j, n // 2)[:, n % 2 * T:(n % 2 + 1) * T])
                    c = [jnp.where(it < 0, y[:R], v) for v in c]
                    ops = jnp.concatenate([_lin(terms, c.__getitem__) for terms in B7], axis=0).astype(BF16)
                    wd[it, pl.ds(7 * po, 7), pl.ds(r // 2, R // 2), :] = pltpu.bitcast(ops, U32).reshape(7, R // 2, T)
                return y

            out = hid.at[:, pl.ds(pl.multiple_of(it * T, T), (15 * NIT + 1) * T)]
            w = {}
            for t in range(NTB):
                order, inner = (UP_ORDER, UP_INNER) if t else (UP_FIRST_ORDER, UP_FIRST_INNER)
                for m in range(2):
                    for po in order:
                        if t == 0:
                            def get(n, j):
                                return load(wt.at[m, n, j], 0, T).astype(F32)

                            c = _outer(B7, po, get)
                            w[m, po] = [_weight_operands(po, pi, c.__getitem__, functools.partial(get, 4))
                                        for pi in range(7)]
                        c = x_products(t, po, w[m, po].__getitem__, inner,
                                       parker(tmp, lambda k: UK(t, m, po, k)), down_operands)
                        done, later = _completion(order, po)
                        for i, v in enumerate(c):
                            if later:
                                store(tmp, UP(t, m, i, po), v)
                            for o in done:
                                y = _lin(C7[o], lambda q: v if q == po else load(tmp, UP(t, m, i, q), T))
                                if m == 0:
                                    store(tmp, UG(t, o, i), jnp.maximum(y, 0.0))
                                else:
                                    j, k = _blk(o, i)
                                    out[t, pl.ds((4 * j + k) * NIT * T, T), :] = load(tmp, UG(t, o, i), T) * y
            assert not jobs
            for k in range(ATT):
                attention_tile(ATT0 + it * ATT + k, ATT0 + k < NG)
            transpose_gate_up(jnp.minimum(it + 1, NIT - 1))
            return carry

        def down_step(t, carry):
            def hidden(j, k):
                return hid[t, pl.ds((4 * j + k) * NIT * T, NIT * T), :]

            def heads(j, k):
                return load(attn.at[4 * t + j], k * T, T if k < 4 else HT).astype(F32)

            count = [0]
            for n, po in enumerate(DOWN_ORDER):
                staged = len(A7[po]) > 1
                for c, source in ((0, hidden), (NIT, heads))[1 - staged:]:
                    for i, v in enumerate(_outer(A7, po, source)):
                        store(tmp, DA(n, i, c), v)
                for i, v in enumerate(_outer(B7, po, lambda k, j: wot[k, pl.ds(j * DQ, DQ), :])):
                    store(tmp, DW(n, i), v)
                done, later = _completion(DOWN_ORDER, po)

                def product(pi):
                    if po == DOWN_ORDER[-1] and pi == int(DOWN_INNER[po in TAIL].replace('k', '')[3]):
                        for o in range(4):
                            if o not in done:
                                o_start(t, o)

                    h = _lin(A7[pi], lambda i: load(tmp, DA(n, i, 0), NIT * T) if staged
                             else hidden(*_blk(A7[po][0][1], i)))
                    w = wd[:, 7 * po + pi]
                    y = None
                    for c in range(NIT):
                        v = _dot(pltpu.bitcast(w[c], BF16), h[c * T:(c + 1) * T].astype(BF16))
                        y = v if y is None else y + v
                        count[0] += 1
                        if count[0] % 4 == 0:
                            y = parker(tmp, DS)(count[0] // 4, y)
                    count[0] += 1
                    w = _weight_operands(po, pi, lambda i: load(tmp, DW(n, i), DQ),
                                         lambda j: wot[4, pl.ds(j * DQ, DQ), :])
                    return y + _product(
                        w, lambda r, rows: _lin(A7[pi], lambda i: load(tmp, DA(n, i, NIT) + r, rows)).astype(BF16),
                        lambda: _tail_operand(po, pi, lambda j: heads(j, 4)).astype(BF16))

                c = _combine(product, DOWN_INNER[po in TAIL], parker(tmp, lambda k: DK(po, k)))
                if later:
                    for i, v in enumerate(c):
                        store(tmp, DP(i, po), v)
                for o in done:
                    for jj in range(2):
                        y = [_lin(C7[o], lambda q: c[i] if q == po else load(tmp, DP(i, q), DQ)) for i in (jj, 2 + jj)]
                        ix = (t, pl.ds((o % 2 * 2 + jj) * DQ, DQ), pl.ds(o // 2 * 2 * T, 2 * T))
                        xo[ix] = (jnp.concatenate(y, axis=1) + xo[ix].astype(F32)).astype(BF16)
            for o in done:
                o_start(t, o)
            return carry

        lax.fori_loop(0, NIT, up_step, 0)
        lax.fori_loop(0, NTB, down_step, 0)
        for t in range(NTB):
            pltpu.make_async_copy(xo.at[t], xo.at[t], sem_o.at[t]).wait()

    scratch = [
        pltpu.VMEM((NTB, D, TB), BF16),
        pltpu.VMEM((D, 3 * D), BF16),
        pltpu.VMEM((D, D), BF16),
        pltpu.VMEM((3 * NIT, D, FC), BF16),
        pltpu.VMEM((NTB, x_arena.size // 2, T), U32),
        pltpu.VMEM((q_arena.size // 2, T), U32),
        pltpu.VMEM((50, (DQ + _split(DQ)) // 2, T), U32),
        pltpu.VMEM((2, 5, 4, HT, T), U32),
        pltpu.VMEM((NIT, 52, DQ // 2, T), U32),
        pltpu.VMEM((5, D, T), F32),
        pltpu.VMEM((f_arena.size, T), F32),
        pltpu.VMEM((NTB, NIT * 16 * T, T), F32),
        pltpu.VMEM(((NTILE + 1) * NG, -(-3 * DQ // 32) * 32, T), F32),
        pltpu.VMEM((NTILE, D // 2, T), U32),
        pltpu.SemaphoreType.DMA((NTB,)),
        pltpu.SemaphoreType.DMA((2,)),
        pltpu.SemaphoreType.DMA((6,)),
        pltpu.SemaphoreType.DMA((NTB,)),
    ]
    return kernel, scratch


@jax.jit
def pallas_parallel_sum__sliding_local_dilated__glu_gated_reglu__prompt_kernel(
    A_x: jax.Array,
    A_wqkv: jax.Array,
    A_wo: jax.Array,
    B_x: jax.Array,
    B_W_gate: jax.Array,
    B_W_up: jax.Array,
    B_W_down: jax.Array,
):
    del B_x
    B, S, D = A_x.shape
    kernel, scratch = _make_kernel(S, D, B_W_gate.shape[1])
    hbm = pl.BlockSpec(memory_space=pl.ANY)
    out = pl.pallas_call(
        kernel,
        out_shape=jax.ShapeDtypeStruct((D, S), A_x.dtype),
        in_specs=[hbm] * 6,
        out_specs=hbm,
        scratch_shapes=scratch,
        compiler_params=pltpu.CompilerParams(vmem_limit_bytes=127 * 2**20),
        name="fused_block",
    )(A_x.reshape(S, D).T, A_wqkv, A_wo, B_W_gate, B_W_up, B_W_down.T)
    return out.T.reshape(B, S, D)
```
